```python
import os as _os
_os.environ.setdefault("JAX_PLATFORMS", "cpu")
import jax
import jax.numpy as jnp

def _softmax(x, axis=-1):
    return jax.nn.softmax(x, axis=axis)
def _gelu(x):
    return jax.nn.gelu(x, approximate=True)
def _silu(x):
    return jax.nn.silu(x)
def _sigmoid(x):
    return jax.nn.sigmoid(x)
def _layernorm(x, axis=-1, eps=1e-5):
    m = jnp.mean(x, axis=axis, keepdims=True)
    v = jnp.var(x, axis=axis, keepdims=True)
    return (x - m) / jnp.sqrt(v + eps)
def _scatter_add(tgt, idx, src, axis=0):
    return tgt.at[idx].add(src)
def _segment_sum(src, seg, n):
    return jax.ops.segment_sum(src, seg, n)
class _Rng:
    def __init__(self, key):
        self._k = key
    def _next(self):
        self._k, sub = jax.random.split(self._k)
        return sub
    def normal(self, shape):
        return jax.random.normal(self._next(), shape, dtype=jnp.bfloat16)
    def randint(self, lo, hi, shape):
        return jax.random.randint(self._next(), shape, lo, hi, dtype=jnp.int32)
    def uniform(self, shape, lo=0.0, hi=1.0):
        return jax.random.uniform(self._next(), shape, jnp.bfloat16, lo, hi)
    def permutation(self, n):
        return jax.random.permutation(self._next(), n)


kernel_name = 'concat_heads__mha_block_cached__mha_block_cached__near_ridge'

def setup_inputs():
    _rng = _Rng(jax.random.key(int.from_bytes(__import__("os").urandom(4), "little")))
    _w = (lambda a: (lambda t: t.astype(jnp.bfloat16) if jnp.issubdtype(t.dtype, jnp.floating) else t)(jnp.asarray(a)))
    def _A_setup():
        B, Sq, D = 32, 32, 640
        H, Sk, Dh = 32, 32, 128
        return {
            "x": _w((lambda *s: _rng.normal(s) * 0.8)(B, Sq, D)),
            "k_cache": _w((lambda *s: _rng.normal(s) * 0.8)(B, H, Sk, Dh)),
            "v_cache": _w((lambda *s: _rng.normal(s) * 0.05)(B, H, Sk, Dh)),
            "wq": _w((lambda *s: _rng.normal(s) * 0.8)(D, H * Dh) * (D ** -0.5)),
            "wo": _w((lambda *s: _rng.normal(s) * 0.05)(H * Dh, D) * ((H * Dh) ** -0.5)),
        }
    _A_in = _A_setup()

    def _B_setup():
        B, Sq, D = 32, 32, 640
        H, Sk, Dh = 32, 32, 128
        return {
            "x": _w((lambda *s: _rng.normal(s) * 0.8)(B, Sq, D)),
            "k_cache": _w((lambda *s: _rng.normal(s) * 0.8)(B, H, Sk, Dh)),
            "v_cache": _w((lambda *s: _rng.normal(s) * 0.05)(B, H, Sk, Dh)),
            "wq": _w((lambda *s: _rng.normal(s) * 0.8)(D, H * Dh) * (D ** -0.5)),
            "wo": _w((lambda *s: _rng.normal(s) * 0.05)(H * Dh, D) * ((H * Dh) ** -0.5)),
        }
    _B_in = _B_setup()

    return {
        "A_x": _A_in["x"],
        "A_k_cache": _A_in["k_cache"],
        "A_v_cache": _A_in["v_cache"],
        "A_wq": _A_in["wq"],
        "A_wo": _A_in["wo"],
        "B_x": _B_in["x"],
        "B_k_cache": _B_in["k_cache"],
        "B_v_cache": _B_in["v_cache"],
        "B_wq": _B_in["wq"],
        "B_wo": _B_in["wo"],
    }

def reference(A_x, A_k_cache, A_v_cache, A_wq, A_wo, B_x, B_k_cache, B_v_cache, B_wq, B_wo):
    def _A_ref(x, k_cache, v_cache, wq, wo):
        B, Sq, D = x.shape
        H, Dh = 32, 128
        q = (lambda x, *d: x.transpose(*d))((x @ wq).reshape(B, Sq, H, Dh), 0, 2, 1, 3)
        scores = jnp.einsum("bhqd,bhkd->bhqk", q, k_cache) * (Dh ** -0.5)
        p = _softmax(scores, axis=-1)
        o = jnp.einsum("bhqk,bhkd->bhqd", p, v_cache)
        return (lambda x, *d: x.transpose(*d))(o, 0, 2, 1, 3).reshape(B, Sq, H * Dh) @ wo

    def _B_ref(x, k_cache, v_cache, wq, wo):
        B, Sq, D = x.shape
        H, Dh = 32, 128
        q = (lambda x, *d: x.transpose(*d))((x @ wq).reshape(B, Sq, H, Dh), 0, 2, 1, 3)
        scores = jnp.einsum("bhqd,bhkd->bhqk", q, k_cache) * (Dh ** -0.5)
        p = _softmax(scores, axis=-1)
        o = jnp.einsum("bhqk,bhkd->bhqd", p, v_cache)
        return (lambda x, *d: x.transpose(*d))(o, 0, 2, 1, 3).reshape(B, Sq, H * Dh) @ wo

    a = _A_ref(A_x, A_k_cache, A_v_cache, A_wq, A_wo)
    b = _B_ref(B_x, B_k_cache, B_v_cache, B_wq, B_wo)
    return jnp.concatenate([a, b], axis=-1)
```

```python
import functools
import jax, jax.numpy as jnp
from jax import lax
import jax.experimental.pallas as pl
import jax.experimental.pallas.tpu as pltpu

B, SQ, D = 32, 32, 640
H, SK, DH = 32, 32, 128
M = B * SQ
SCALE = DH ** -0.5


def make(G=4):
    NG = H // G
    W = G * DH

    def kernel(xa, ka, va, wqa, woa, xb, kb, vb, wqb, wob, out_ref,
               xbuf, wqbuf, kbuf, vbuf, wobuf, obuf, acc, sems, xsem):
        g = pl.program_id(0)
        slot = g % 2
        srcs = ((ka, va, wqa, woa), (kb, vb, wqb, wob))

        def copies(t, gg, sl):
            k, v, wq, wo = srcs[t]
            return [
                pltpu.make_async_copy(wq.at[:, pl.ds(gg * W, W)], wqbuf.at[t, sl], sems.at[t, 0, sl]),
                pltpu.make_async_copy(k.at[:, pl.ds(gg * G, G)], kbuf.at[t, sl], sems.at[t, 1, sl]),
                pltpu.make_async_copy(v.at[:, pl.ds(gg * G, G)], vbuf.at[t, sl], sems.at[t, 2, sl]),
                pltpu.make_async_copy(wo.at[pl.ds(gg * W, W), :], wobuf.at[t, sl], sems.at[t, 3, sl]),
            ]

        def start_all(gg, sl):
            ca = copies(0, gg, sl)
            cb = copies(1, gg, sl)
            for c in (ca[0], ca[1], ca[2], cb[0], cb[1], cb[2], ca[3], cb[3]):
                c.start()

        ca = copies(0, 0, slot)
        cb = copies(1, 0, slot)

        lb = lax.broadcasted_iota(jnp.int32, (32, 128), 1) // 32

        def qproj(t):
            return jnp.dot(xbuf[t], wqbuf[t, slot], preferred_element_type=jnp.float32).astype(jnp.bfloat16)

        def recip(l):
            r0 = pl.reciprocal(l, approx=True)
            return r0 * (2.0 - l * r0)

        def attn(t, q):
            for h in range(G):
                for b4 in range(8):
                    qt = q[b4 * 128:(b4 + 1) * 128, h * DH:(h + 1) * DH]
                    kt = kbuf[t, slot, 4 * b4:4 * b4 + 4, h].reshape(128, DH)
                    vt = vbuf[t, slot, 4 * b4:4 * b4 + 4, h].reshape(128, DH)
                    st = lax.dot_general(kt, qt, (((1,), (1,)), ((), ())),
                                         preferred_element_type=jnp.float32)
                    cc = jnp.where(lb == 0, st[0:32],
                                   jnp.where(lb == 1, st[32:64],
                                             jnp.where(lb == 2, st[64:96], st[96:128])))
                    m = jnp.max(cc, axis=0, keepdims=True)
                    p = jnp.exp((cc - m) * SCALE)
                    l = jnp.sum(p, axis=0, keepdims=True)
                    p = p * recip(l)
                    pt = jnp.concatenate([jnp.where(lb == j, p, 0.0) for j in range(4)], axis=0).astype(jnp.bfloat16)
                    ot = lax.dot_general(pt, vt, (((0,), (0,)), ((), ())),
                                         preferred_element_type=jnp.float32)
                    obuf[t, b4 * 128:(b4 + 1) * 128, h * DH:(h + 1) * DH] = ot.astype(jnp.bfloat16)

        def oproj(t, first):
            y = jnp.dot(obuf[t], wobuf[t, slot], preferred_element_type=jnp.float32)
            if first:
                acc[t] = y
            else:
                acc[t] += y

        @pl.when(g == 0)
        def _():
            cxa = pltpu.make_async_copy(xa, xbuf.at[0], xsem.at[0])
            cxb = pltpu.make_async_copy(xb, xbuf.at[1], xsem.at[1])
            cxa.start(); ca[0].start()
            cxa.wait(); ca[0].wait()
            ca[1].start(); ca[2].start(); cxb.start(); cb[0].start()
            qa = qproj(0)
            ca[1].wait(); ca[2].wait(); cxb.wait(); cb[0].wait()
            cb[1].start(); cb[2].start(); ca[3].start(); cb[3].start()
            attn(0, qa)
            qb = qproj(1)
            cb[1].wait(); cb[2].wait(); ca[3].wait(); cb[3].wait()
            start_all(1, 1)
            attn(1, qb)
            oproj(0, True)
            oproj(1, True)

        @pl.when(g > 0)
        def _():
            for cc in ca + cb:
                cc.wait()

            @pl.when(g + 1 < NG)
            def _():
                start_all(g + 1, 1 - slot)
            qa = qproj(0)
            attn(0, qa)
            qb = qproj(1)
            attn(1, qb)
            oproj(0, False)
            oproj(1, False)

        @pl.when(g == NG - 1)
        def _():
            out_ref[:, :D] = acc[0].astype(out_ref.dtype)
            out_ref[:, D:] = acc[1].astype(out_ref.dtype)

    @jax.jit
    def fn(A_x, A_k, A_v, A_wq, A_wo, B_x, B_k, B_v, B_wq, B_wo):
        xa = A_x.reshape(M, D)
        xb = B_x.reshape(M, D)
        anyspec = pl.BlockSpec(memory_space=pl.ANY)
        out = pl.pallas_call(
            kernel,
            grid=(NG,),
            in_specs=[anyspec] * 10,
            out_specs=pl.BlockSpec((M, 2 * D), lambda s: (0, 0)),
            out_shape=jax.ShapeDtypeStruct((M, 2 * D), jnp.bfloat16),
            scratch_shapes=[
                pltpu.VMEM((2, M, D), jnp.bfloat16),
                pltpu.VMEM((2, 2, D, W), jnp.bfloat16),
                pltpu.VMEM((2, 2, B, G, SK, DH), jnp.bfloat16),
                pltpu.VMEM((2, 2, B, G, SK, DH), jnp.bfloat16),
                pltpu.VMEM((2, 2, W, D), jnp.bfloat16),
                pltpu.VMEM((2, M, W), jnp.bfloat16),
                pltpu.VMEM((2, M, D), jnp.float32),
                pltpu.SemaphoreType.DMA((2, 4, 2)),
                pltpu.SemaphoreType.DMA((2,)),
            ],
            compiler_params=pltpu.CompilerParams(
                dimension_semantics=("arbitrary",),
                vmem_limit_bytes=100 * 1024 * 1024,
            ),
        )(xa, A_k, A_v, A_wq, A_wo, xb, B_k, B_v, B_wq, B_wo)
        return out.reshape(B, SQ, 2 * D)
    return fn


_fn = make(4)


@jax.jit
def pallas_concat_heads__mha_block_cached__mha_block_cached__near_ridge_kernel(
        A_x, A_k_cache, A_v_cache, A_wq, A_wo, B_x, B_k_cache, B_v_cache, B_wq, B_wo):
    return _fn(A_x, A_k_cache, A_v_cache, A_wq, A_wo, B_x, B_k_cache, B_v_cache, B_wq, B_wo)
```

```python
import jax
import jax.numpy as jnp
from jax import lax
import jax.experimental.pallas as pl
import jax.experimental.pallas.tpu as pltpu

B, SQ, D = 32, 32, 640
H, SK, DH = 32, 32, 128
M = B * SQ
SCALE = DH ** -0.5

G = 4
NS = H // G
HALF = NS // 2
W = G * DH
OC = 8
OR = M // OC
RC = 256


def _kernel(xa, ka, va, wqa, woa, xb, kb, vb, wqb, wob, out_hbm,
            xbuf, wqbuf, kbuf, vbuf, wobuf, qbuf, obuf, acc, ostage, pbuf,
            sems, osem):
    g = pl.program_id(0)
    slot = g % 2
    srcs = ((ka, va, wqa, woa), (kb, vb, wqb, wob))

    def copies(t, j, gg, sl):
        k, v, wq, wo = srcs[t]
        return [
            pltpu.make_async_copy(wq.at[:, pl.ds(gg * W, W)], wqbuf.at[j, sl],
                                  sems.at[(j * 4 + 0) * 2 + sl]),
            pltpu.make_async_copy(k.at[:, pl.ds(gg * G, G)], kbuf.at[j, sl],
                                  sems.at[(j * 4 + 1) * 2 + sl]),
            pltpu.make_async_copy(v.at[:, pl.ds(gg * G, G)], vbuf.at[j, sl],
                                  sems.at[(j * 4 + 2) * 2 + sl]),
            pltpu.make_async_copy(wo.at[pl.ds(gg * W, W), :], wobuf.at[j, sl],
                                  sems.at[(j * 4 + 3) * 2 + sl]),
        ]

    def start_step(t, s, sl):
        p0 = copies(t, 0, 2 * s, sl)
        p1 = copies(t, 1, 2 * s + 1, sl)
        for c in (p0[0], p1[0], p0[1], p0[2], p1[1], p1[2], p0[3], p1[3]):
            c.start()

    c0 = copies(0, 0, 0, slot)
    c1 = copies(0, 1, 0, slot)
    cxa = pltpu.make_async_copy(xa, xbuf.at[0], sems.at[16])
    cxb = pltpu.make_async_copy(xb, xbuf.at[1], sems.at[17])

    lb = lax.broadcasted_iota(jnp.int32, (32, 128), 1) // 32

    def qproj(t, j):
        return jnp.dot(xbuf[t], wqbuf[j, slot],
                       preferred_element_type=jnp.float32).astype(jnp.bfloat16)

    def recip(l):
        r0 = pl.reciprocal(l, approx=True)
        return r0 * (2.0 - l * r0)

    def attn_qk(j, q):
        for h in range(G):
            for b4 in range(8):
                qt = q[b4 * 128:(b4 + 1) * 128, h * DH:(h + 1) * DH]
                kt = kbuf[j, slot, 4 * b4:4 * b4 + 4, h].reshape(128, DH)
                st = lax.dot_general(kt, qt, (((1,), (1,)), ((), ())),
                                     preferred_element_type=jnp.float32)
                cc = jnp.where(lb == 0, st[0:32],
                               jnp.where(lb == 1, st[32:64],
                                         jnp.where(lb == 2, st[64:96], st[96:128])))
                m = jnp.max(cc, axis=0, keepdims=True)
                p = jnp.exp((cc - m) * SCALE)
                l = jnp.sum(p, axis=0, keepdims=True)
                pbuf[j, h * 8 + b4] = p * recip(l)

    def attn_pv(j):
        for h in range(G):
            for b4 in range(8):
                vt = vbuf[j, slot, 4 * b4:4 * b4 + 4, h].reshape(128, DH)
                p = pbuf[j, h * 8 + b4]
                pt = jnp.concatenate([jnp.where(lb == i, p, 0.0) for i in range(4)],
                                     axis=0).astype(jnp.bfloat16)
                ot = lax.dot_general(pt, vt, (((0,), (0,)), ((), ())),
                                     preferred_element_type=jnp.float32)
                obuf[j, b4 * 128:(b4 + 1) * 128, h * DH:(h + 1) * DH] = ot.astype(jnp.bfloat16)

    def oproj(t, j, first=False):
        y = jnp.dot(obuf[j], wobuf[j, slot], preferred_element_type=jnp.float32)
        if first:
            acc[t] = y
        else:
            acc[t] += y

    def ocopy(t, c):
        return pltpu.make_async_copy(ostage.at[t, pl.ds(c * OR, OR)],
                                     out_hbm.at[pl.ds(c * OR, OR), pl.ds(t * D, D)],
                                     osem.at[t, c])

    s0a = copies(0, 0, 0, 0)
    s0b = copies(0, 1, 1, 0)
    s1a = copies(0, 0, 2, 1)
    s1b = copies(0, 1, 3, 1)
    first_copies = (cxa, s0a[0], s0b[0], s0a[1], s0a[2], s0b[1], s0b[2], s0a[3], s0b[3],
                    s1a[0], s1b[0], s1a[1], s1a[2], s1b[1], s1b[2], s1a[3], s1b[3], cxb)
    for c in first_copies:
        pl.when(g == 0)(c.start)

    @pl.when(g == 0)
    def _():
        acc[1] = jnp.zeros((M, D), jnp.float32)

        def q_body(c, carry):
            rows = pl.ds(pl.multiple_of(c * RC, RC), RC)
            qbuf[rows] = jnp.dot(xbuf[0, rows], wqbuf[0, slot],
                                 preferred_element_type=jnp.float32).astype(jnp.bfloat16)
            return carry

        def o_body(c, carry):
            rows = pl.ds(pl.multiple_of(c * RC, RC), RC)
            acc[0, rows] += jnp.dot(obuf[1, rows], wobuf[1, slot],
                                    preferred_element_type=jnp.float32)
            return carry

        cxa.wait()
        c0[0].wait()
        lax.fori_loop(0, M // RC, q_body, 0)
        c1[0].wait()
        c0[1].wait()
        attn_qk(0, qbuf[...])
        q1 = qproj(0, 1)
        c0[2].wait()
        c1[1].wait()
        attn_pv(0)
        attn_qk(1, q1)
        c1[2].wait()
        c0[3].wait()
        c1[3].wait()
        oproj(0, 0, first=True)
        attn_pv(1)
        lax.fori_loop(0, M // RC, o_body, 0)

    @pl.when(jnp.logical_and(g > 0, g < NS - 1))
    def _():
        t = g // HALF
        for cc in c0 + c1:
            cc.wait()

        @pl.when(g == HALF)
        def _():
            cxb.wait()

        @pl.when(g + 1 < HALF)
        def _():
            start_step(0, g + 1, 1 - slot)

        @pl.when(g + 1 >= HALF)
        def _():
            start_step(1, g + 1 - HALF, 1 - slot)

        q0 = qproj(t, 0)
        attn_qk(0, q0)
        q1 = qproj(t, 1)
        attn_pv(0)
        attn_qk(1, q1)
        oproj(t, 0)
        attn_pv(1)
        oproj(t, 1)

    @pl.when(g == NS - 1)
    def _():
        for cc in c0 + c1:
            cc.wait()
        for c in range(OC):
            rows = pl.ds(c * OR, OR)
            ostage[0, rows] = acc[0, rows].astype(jnp.bfloat16)
            ocopy(0, c).start()
        q0 = qproj(1, 0)
        attn_qk(0, q0)
        q1 = qproj(1, 1)
        attn_pv(0)
        attn_qk(1, q1)
        oproj(1, 0)
        attn_pv(1)
        for c in range(OC):
            rows = pl.ds(c * OR, OR)
            y = jnp.dot(obuf[1, rows], wobuf[1, slot], preferred_element_type=jnp.float32)
            ostage[1, rows] = (acc[1, rows] + y).astype(jnp.bfloat16)
            ocopy(1, c).start()
        for t in range(2):
            for c in range(OC):
                ocopy(t, c).wait()


@jax.jit
def pallas_concat_heads__mha_block_cached__mha_block_cached__near_ridge_kernel(
    A_x: jax.Array,
    A_k_cache: jax.Array,
    A_v_cache: jax.Array,
    A_wq: jax.Array,
    A_wo: jax.Array,
    B_x: jax.Array,
    B_k_cache: jax.Array,
    B_v_cache: jax.Array,
    B_wq: jax.Array,
    B_wo: jax.Array,
):
    xa = A_x.reshape(M, D)
    xb = B_x.reshape(M, D)
    anyspec = pl.BlockSpec(memory_space=pl.ANY)
    out = pl.pallas_call(
        _kernel,
        grid=(NS,),
        in_specs=[anyspec] * 10,
        out_specs=anyspec,
        out_shape=jax.ShapeDtypeStruct((M, 2 * D), jnp.bfloat16),
        scratch_shapes=[
            pltpu.VMEM((2, M, D), jnp.bfloat16),
            pltpu.VMEM((2, 2, D, W), jnp.bfloat16),
            pltpu.VMEM((2, 2, B, G, SK, DH), jnp.bfloat16),
            pltpu.VMEM((2, 2, B, G, SK, DH), jnp.bfloat16),
            pltpu.VMEM((2, 2, W, D), jnp.bfloat16),
            pltpu.VMEM((M, W), jnp.bfloat16),
            pltpu.VMEM((2, M, W), jnp.bfloat16),
            pltpu.VMEM((2, M, D), jnp.float32),
            pltpu.VMEM((2, M, D), jnp.bfloat16),
            pltpu.VMEM((2, G * 8, 32, 128), jnp.float32),
            pltpu.SemaphoreType.DMA((18,)),
            pltpu.SemaphoreType.DMA((2, OC)),
        ],
        compiler_params=pltpu.CompilerParams(
            dimension_semantics=("arbitrary",),
            vmem_limit_bytes=100 * 1024 * 1024,
            disable_bounds_checks=True,
        ),
    )(xa, A_k_cache, A_v_cache, A_wq, A_wo, xb, B_k_cache, B_v_cache, B_wq, B_wo)
    return out.reshape(B, SQ, 2 * D)
```

```python
import jax
import jax.numpy as jnp
from jax import lax
import jax.experimental.pallas as pl
import jax.experimental.pallas.tpu as pltpu

B, SQ, D = 32, 32, 640
H, SK, DH = 32, 32, 128
M = B * SQ
SCALE = DH ** -0.5

G = 4
NS = H // G
HALF = NS // 2
W = G * DH
OC = 8
OR = M // OC
RC = 256


def _kernel(xa, ka, va, wqa, woa, xb, kb, vb, wqb, wob, out_hbm,
            xbuf, wqbuf, kbuf, vbuf, wobuf, qbuf, obuf, acc, ostage, pbuf,
            sems, osem):
    g = pl.program_id(0)
    slot = g % 2
    srcs = ((ka, va, wqa, woa), (kb, vb, wqb, wob))

    def copies(t, j, gg, sl):
        k, v, wq, wo = srcs[t]
        return [
            pltpu.make_async_copy(wq.at[:, pl.ds(gg * W, W)], wqbuf.at[j, sl],
                                  sems.at[(j * 4 + 0) * 2 + sl]),
            pltpu.make_async_copy(k.at[:, pl.ds(gg * G, G)], kbuf.at[j, sl],
                                  sems.at[(j * 4 + 1) * 2 + sl]),
            pltpu.make_async_copy(v.at[:, pl.ds(gg * G, G)], vbuf.at[j, sl],
                                  sems.at[(j * 4 + 2) * 2 + sl]),
            pltpu.make_async_copy(wo.at[pl.ds(gg * W, W), :], wobuf.at[j, sl],
                                  sems.at[(j * 4 + 3) * 2 + sl]),
        ]

    def start_step(t, s, sl):
        p0 = copies(t, 0, 2 * s, sl)
        p1 = copies(t, 1, 2 * s + 1, sl)
        for c in (p0[0], p1[0], p0[1], p0[2], p1[1], p1[2], p0[3], p1[3]):
            c.start()

    c0 = copies(0, 0, 0, slot)
    c1 = copies(0, 1, 0, slot)
    cxa = pltpu.make_async_copy(xa, xbuf.at[0], sems.at[16])
    cxb = pltpu.make_async_copy(xb, xbuf.at[1], sems.at[17])

    lb = lax.broadcasted_iota(jnp.int32, (32, 128), 1) // 32

    def qproj(t, j):
        return jnp.dot(xbuf[t], wqbuf[j, slot],
                       preferred_element_type=jnp.float32).astype(jnp.bfloat16)

    def recip(l):
        r0 = pl.reciprocal(l, approx=True)
        return r0 * (2.0 - l * r0)

    def attn_qk(j, q):
        for h in range(G):
            for b4 in range(8):
                qt = q[b4 * 128:(b4 + 1) * 128, h * DH:(h + 1) * DH]
                kt = kbuf[j, slot, 4 * b4:4 * b4 + 4, h].reshape(128, DH)
                st = lax.dot_general(kt, qt, (((1,), (1,)), ((), ())),
                                     preferred_element_type=jnp.float32)
                cc = jnp.where(lb == 0, st[0:32],
                               jnp.where(lb == 1, st[32:64],
                                         jnp.where(lb == 2, st[64:96], st[96:128])))
                m = jnp.max(cc, axis=0, keepdims=True)
                p = jnp.exp((cc - m) * SCALE)
                l = jnp.sum(p, axis=0, keepdims=True)
                pbuf[j, h * 8 + b4] = p * recip(l)

    def attn_pv(j):
        for h in range(G):
            for b4 in range(8):
                vt = vbuf[j, slot, 4 * b4:4 * b4 + 4, h].reshape(128, DH)
                p = pbuf[j, h * 8 + b4]
                pt = jnp.concatenate([jnp.where(lb == i, p, 0.0) for i in range(4)],
                                     axis=0).astype(jnp.bfloat16)
                ot = lax.dot_general(pt, vt, (((0,), (0,)), ((), ())),
                                     preferred_element_type=jnp.float32)
                obuf[j, b4 * 128:(b4 + 1) * 128, h * DH:(h + 1) * DH] = ot.astype(jnp.bfloat16)

    def oproj(t, j):
        acc[t] += jnp.dot(obuf[j], wobuf[j, slot], preferred_element_type=jnp.float32)

    def ocopy(t, c):
        return pltpu.make_async_copy(ostage.at[t, pl.ds(c * OR, OR)],
                                     out_hbm.at[pl.ds(c * OR, OR), pl.ds(t * D, D)],
                                     osem.at[t, c])

    s0a = copies(0, 0, 0, 0)
    s0b = copies(0, 1, 1, 0)
    s1a = copies(0, 0, 2, 1)
    s1b = copies(0, 1, 3, 1)
    first_copies = (cxa, s0a[0], s0b[0], s0a[1], s0a[2], s0b[1], s0b[2], s0a[3], s0b[3],
                    s1a[0], s1b[0], s1a[1], s1a[2], s1b[1], s1b[2], s1a[3], s1b[3], cxb)
    for c in first_copies:
        pl.when(g == 0)(c.start)

    @pl.when(g == 0)
    def _():
        acc[1] = jnp.zeros((M, D), jnp.float32)

        def q_body(c, carry):
            rows = pl.ds(pl.multiple_of(c * RC, RC), RC)
            qbuf[rows] = jnp.dot(xbuf[0, rows], wqbuf[0, slot],
                                 preferred_element_type=jnp.float32).astype(jnp.bfloat16)
            return carry

        def o_body(c, carry):
            rows = pl.ds(pl.multiple_of(c * RC, RC), RC)
            acc[0, rows] = (jnp.dot(obuf[0, rows], wobuf[0, slot],
                                    preferred_element_type=jnp.float32)
                            + jnp.dot(obuf[1, rows], wobuf[1, slot],
                                      preferred_element_type=jnp.float32))
            return carry

        cxa.wait()
        c0[0].wait()
        lax.fori_loop(0, M // RC, q_body, 0)
        c1[0].wait()
        c0[1].wait()
        attn_qk(0, qbuf[...])
        q1 = qproj(0, 1)
        c0[2].wait()
        c1[1].wait()
        attn_pv(0)
        attn_qk(1, q1)
        c1[2].wait()
        c0[3].wait()
        c1[3].wait()
        attn_pv(1)
        lax.fori_loop(0, M // RC, o_body, 0)

    @pl.when(jnp.logical_and(g > 0, g < NS - 1))
    def _():
        t = g // HALF
        for cc in c0 + c1:
            cc.wait()

        @pl.when(g == HALF)
        def _():
            cxb.wait()

        @pl.when(g + 1 < HALF)
        def _():
            start_step(0, g + 1, 1 - slot)

        @pl.when(g + 1 >= HALF)
        def _():
            start_step(1, g + 1 - HALF, 1 - slot)

        q0 = qproj(t, 0)
        attn_qk(0, q0)
        q1 = qproj(t, 1)
        attn_pv(0)
        attn_qk(1, q1)
        oproj(t, 0)
        attn_pv(1)
        oproj(t, 1)

    @pl.when(g == NS - 1)
    def _():
        for cc in c0 + c1:
            cc.wait()
        for c in range(OC):
            rows = pl.ds(c * OR, OR)
            ostage[0, rows] = acc[0, rows].astype(jnp.bfloat16)
            ocopy(0, c).start()
        q0 = qproj(1, 0)
        attn_qk(0, q0)
        q1 = qproj(1, 1)
        attn_pv(0)
        attn_qk(1, q1)
        oproj(1, 0)
        attn_pv(1)
        for c in range(OC):
            rows = pl.ds(c * OR, OR)
            y = jnp.dot(obuf[1, rows], wobuf[1, slot], preferred_element_type=jnp.float32)
            ostage[1, rows] = (acc[1, rows] + y).astype(jnp.bfloat16)
            ocopy(1, c).start()
        for t in range(2):
            for c in range(OC):
                ocopy(t, c).wait()


@jax.jit
def pallas_concat_heads__mha_block_cached__mha_block_cached__near_ridge_kernel(
    A_x: jax.Array,
    A_k_cache: jax.Array,
    A_v_cache: jax.Array,
    A_wq: jax.Array,
    A_wo: jax.Array,
    B_x: jax.Array,
    B_k_cache: jax.Array,
    B_v_cache: jax.Array,
    B_wq: jax.Array,
    B_wo: jax.Array,
):
    xa = A_x.reshape(M, D)
    xb = B_x.reshape(M, D)
    anyspec = pl.BlockSpec(memory_space=pl.ANY)
    out = pl.pallas_call(
        _kernel,
        grid=(NS,),
        in_specs=[anyspec] * 10,
        out_specs=anyspec,
        out_shape=jax.ShapeDtypeStruct((M, 2 * D), jnp.bfloat16),
        scratch_shapes=[
            pltpu.VMEM((2, M, D), jnp.bfloat16),
            pltpu.VMEM((2, 2, D, W), jnp.bfloat16),
            pltpu.VMEM((2, 2, B, G, SK, DH), jnp.bfloat16),
            pltpu.VMEM((2, 2, B, G, SK, DH), jnp.bfloat16),
            pltpu.VMEM((2, 2, W, D), jnp.bfloat16),
            pltpu.VMEM((M, W), jnp.bfloat16),
            pltpu.VMEM((2, M, W), jnp.bfloat16),
            pltpu.VMEM((2, M, D), jnp.float32),
            pltpu.VMEM((2, M, D), jnp.bfloat16),
            pltpu.VMEM((2, G * 8, 32, 128), jnp.float32),
            pltpu.SemaphoreType.DMA((18,)),
            pltpu.SemaphoreType.DMA((2, OC)),
        ],
        compiler_params=pltpu.CompilerParams(
            dimension_semantics=("arbitrary",),
            vmem_limit_bytes=100 * 1024 * 1024,
            disable_bounds_checks=True,
        ),
    )(xa, A_k_cache, A_v_cache, A_wq, A_wo, xb, B_k_cache, B_v_cache, B_wq, B_wo)
    return out.reshape(B, SQ, 2 * D)
```
